```python
import os as _os
_os.environ.setdefault("JAX_PLATFORMS", "cpu")
import jax
import jax.numpy as jnp

def _softmax(x, axis=-1):
    return jax.nn.softmax(x, axis=axis)
def _gelu(x):
    return jax.nn.gelu(x, approximate=True)
def _silu(x):
    return jax.nn.silu(x)
def _sigmoid(x):
    return jax.nn.sigmoid(x)
def _layernorm(x, axis=-1, eps=1e-5):
    m = jnp.mean(x, axis=axis, keepdims=True)
    v = jnp.var(x, axis=axis, keepdims=True)
    return (x - m) / jnp.sqrt(v + eps)
def _scatter_add(tgt, idx, src, axis=0):
    return tgt.at[idx].add(src)
def _segment_sum(src, seg, n):
    return jax.ops.segment_sum(src, seg, n)
class _Rng:
    def __init__(self, key):
        self._k = key
    def _next(self):
        self._k, sub = jax.random.split(self._k)
        return sub
    def normal(self, shape):
        return jax.random.normal(self._next(), shape, dtype=jnp.bfloat16)
    def randint(self, lo, hi, shape):
        return jax.random.randint(self._next(), shape, lo, hi, dtype=jnp.int32)
    def uniform(self, shape, lo=0.0, hi=1.0):
        return jax.random.uniform(self._next(), shape, jnp.bfloat16, lo, hi)
    def permutation(self, n):
        return jax.random.permutation(self._next(), n)


kernel_name = 'gated_mix__ssm_conv_s5__glu_gated_geglu__prompt'

def setup_inputs():
    _rng = _Rng(jax.random.key(int.from_bytes(__import__("os").urandom(4), "little")))
    _w = (lambda a: (lambda t: t.astype(jnp.bfloat16) if jnp.issubdtype(t.dtype, jnp.floating) else t)(jnp.asarray(a)))
    def _A_setup():
        B, S, D = 1, 2048, 448
        P = D
        Lambda_re = -0.5 * jnp.exp((lambda *s: _rng.normal(s) * 0.4)(P))
        Lambda_im = (lambda *s: _rng.normal(s) * 0.4)(P) * 1.0
        B_re = (lambda *s: _rng.normal(s) * 0.4)(P, D) * (D ** -0.5)
        B_im = (lambda *s: _rng.normal(s) * 0.4)(P, D) * (D ** -0.5)
        C_re = (lambda *s: _rng.normal(s) * 0.4)(D, P) * (P ** -0.5)
        C_im = (lambda *s: _rng.normal(s) * 0.4)(D, P) * (P ** -0.5)
        log_dt = (lambda *s: _rng.normal(s) * 0.4)(P) * 0.3 - 2.0
        Dskip = (lambda *s: _rng.normal(s) * 0.4)(D)
        return {
            "x": _w((lambda *s: _rng.normal(s) * 0.05)(B, S, D)),
            "Lambda_re": _w(Lambda_re),
            "Lambda_im": _w(Lambda_im),
            "B_re": _w(B_re),
            "B_im": _w(B_im),
            "C_re": _w(C_re),
            "C_im": _w(C_im),
            "log_dt": _w(log_dt),
            "Dskip": _w(Dskip),
        }
    _A_in = _A_setup()

    def _B_setup():
        B, S, Dm, Df = 1, 2048, 448, 1792
        return {
            "x": _w((lambda *s: _rng.normal(s) * 0.05)(B, S, Dm)),
            "w_gate": _w((lambda *s: _rng.normal(s) * 1.6)(Dm, Df) * (Dm ** -0.5)),
            "w_up": _w((lambda *s: _rng.normal(s) * 1.6)(Dm, Df) * (Dm ** -0.5)),
            "w_down": _w((lambda *s: _rng.normal(s) * 1.6)(Df, Dm) * (Df ** -0.5)),
        }
    _B_in = _B_setup()

    return {
        "A_x": _A_in["x"],
        "A_Lambda_re": _A_in["Lambda_re"],
        "A_Lambda_im": _A_in["Lambda_im"],
        "A_B_re": _A_in["B_re"],
        "A_B_im": _A_in["B_im"],
        "A_C_re": _A_in["C_re"],
        "A_C_im": _A_in["C_im"],
        "A_log_dt": _A_in["log_dt"],
        "A_Dskip": _A_in["Dskip"],
        "B_x": _B_in["x"],
        "B_w_gate": _B_in["w_gate"],
        "B_w_up": _B_in["w_up"],
        "B_w_down": _B_in["w_down"],
        "gate_w": _w((lambda *s: _rng.normal(s) * 0.05)(448) * 16.0),
    }

def reference(A_x, A_Lambda_re, A_Lambda_im, A_B_re, A_B_im, A_C_re, A_C_im, A_log_dt, A_Dskip, B_x, B_w_gate, B_w_up, B_w_down, gate_w):
    def _A_ref(x, Lambda_re, Lambda_im, B_re, B_im, C_re, C_im, log_dt, Dskip):
        Bsz, L, H = x.shape
        Lam = Lambda_re + 1j * Lambda_im
        Bmat = B_re + 1j * B_im
        Cmat = C_re + 1j * C_im
        dt = jnp.exp(log_dt)
        Lam_bar = jnp.exp(dt * Lam)
        B_bar = ((Lam_bar - 1.0) / Lam)[:, None] * Bmat
        Bu = jnp.einsum("bld,pd->blp", x + 0j, B_bar)
        h = jnp.zeros_like(Bu[:, 0, :])
        hs = []
        for t in range(L):
            h = Lam_bar[None, :] * h + Bu[:, t, :]
            hs.append(h)
        hseq = jnp.stack(hs, 1)
        y = 2.0 * jnp.einsum("blp,dp->bld", hseq, Cmat).real + x * Dskip[None, None, :]
        return y

    def _B_ref(x, w_gate, w_up, w_down):
        g = jnp.einsum("bsd,df->bsf", x, w_gate)
        u = jnp.einsum("bsd,df->bsf", x, w_up)
        h = _gelu(g) * u
        return jnp.einsum("bsf,fd->bsd", h, w_down)

    x = A_x
    g = _sigmoid((x * gate_w).sum(-1, keepdims=True))
    a = _A_ref(x, A_Lambda_re, A_Lambda_im, A_B_re, A_B_im, A_C_re, A_C_im, A_log_dt, A_Dskip)
    b = _B_ref(x, B_w_gate, B_w_up, B_w_down)
    return g * a + (1 - g) * b
```

```python
import jax
import jax.numpy as jnp
from jax import lax
import jax.experimental.pallas as pl
import jax.experimental.pallas.tpu as pltpu

NT = (((1,), (1,)), ((), ()))
NN = (((1,), (0,)), ((), ()))
f32 = jnp.float32
bf16 = jnp.bfloat16
D = 448; F = 1792; S = 2048; LT = 128; H = 64


def cmul(ar, ai, br, bi):
    return ar * br - ai * bi, ar * bi + ai * br


def prep_params(lre_ref, lim_ref, ldt_ref, dsk_ref, gw_ref, cre_ref, cim_ref, ccat_ref, lam_ref, pw_ref, dcol_ref, gcol_ref, Tc):
    lre = lre_ref[...].astype(f32)[None, :]
    lim = lim_ref[...].astype(f32)[None, :]
    dt = jnp.exp(ldt_ref[...].astype(f32)).astype(bf16).astype(f32)[None, :]
    mag = jnp.exp(dt * lre)
    ang = dt * lim
    br = mag * jnp.cos(ang)
    bi = mag * jnp.sin(ang)
    nr = br - 1.0
    ni = bi
    big = jnp.abs(lre) >= jnp.abs(lim)
    num = jnp.where(big, lim, lre)
    den = jnp.where(big, lre, lim)
    r = num / den
    dd = den + num * r
    cr = jnp.where(big, nr + ni * r, nr * r + ni) / dd
    ci = jnp.where(big, ni - nr * r, ni * r - nr) / dd
    cr = 2.0 * cr
    ci = 2.0 * ci
    cre = cre_ref[...].astype(f32)
    cim = cim_ref[...].astype(f32)
    pr = cre * cr - cim * ci
    pi = -(cre * ci + cim * cr)
    ccat_ref[:, 0:384] = pr[:, 0:384].astype(bf16)
    ccat_ref[:, 384:512] = jnp.concatenate([pr[:, 384:448], pi[:, 384:448]], axis=1).astype(bf16)
    ccat_ref[:, 512:896] = pi[:, 0:384].astype(bf16)
    def tiles(v, sign):
        t3 = jnp.concatenate([v[:, 384:448], sign * v[:, 384:448]], axis=1)
        return jnp.stack([v[:, 0:128], v[:, 128:256], v[:, 256:384], t3], axis=0)
    Lr = jnp.broadcast_to(tiles(br, 1.0), (4, 8, LT))
    Li = jnp.broadcast_to(tiles(bi, -1.0), (4, 8, LT))
    lam_ref[0] = Lr
    lam_ref[1] = Li
    sub = lax.broadcasted_iota(jnp.int32, (4, 8, LT), 1) + 1
    qr = jnp.ones((4, 8, LT), f32)
    qi = jnp.zeros((4, 8, LT), f32)
    sr, si = Lr, Li
    for b in range(4):
        tr_, ti_ = cmul(qr, qi, sr, si)
        m = ((sub >> b) & 1) == 1
        qr = jnp.where(m, tr_, qr)
        qi = jnp.where(m, ti_, qi)
        if b < 3:
            sr, si = cmul(sr, si, sr, si)
    l8r, l8i = sr, si
    for blk in range(Tc // 8):
        pw_ref[0, :, blk * 8:(blk + 1) * 8, :] = qr
        pw_ref[1, :, blk * 8:(blk + 1) * 8, :] = qi
        if blk + 1 < Tc // 8:
            qr, qi = cmul(qr, qi, l8r, l8i)
    ar, ai = l8r, l8i
    n = 8
    while n < Tc:
        ar, ai = cmul(ar, ai, ar, ai)
        n *= 2
    for s in range(3):
        lam_ref[2 + 2 * s] = ar
        lam_ref[3 + 2 * s] = ai
        if s < 2:
            ar, ai = cmul(ar, ai, ar, ai)
    dsk = dsk_ref[...].astype(f32)[None, :]
    gw = gw_ref[...].astype(f32)[None, :]
    dcol_ref[...] = jnp.broadcast_to(dsk, (LT, D)).T
    gcol_ref[...] = jnp.broadcast_to(gw, (LT, D)).T


def ssm_in(x, bre_ref, bim_ref, u_ref, tm, Tc):
    st = Tc + 1
    def put(k, val):
        for c in range(8):
            u_ref[k, pl.ds(c * st, Tc), :] = val[c * Tc:(c + 1) * Tc, :]
    for k in range(3):
        put(k, lax.dot_general(x, bre_ref[k * LT:(k + 1) * LT, :], NT, preferred_element_type=f32))
        put(4 + k, lax.dot_general(x, bim_ref[k * LT:(k + 1) * LT, :], NT, preferred_element_type=f32))
    bm = jnp.concatenate([bre_ref[384:448, :], bim_ref[384:448, :]], axis=0)
    um = lax.dot_general(x, bm, NT, preferred_element_type=f32)
    put(3, um)
    put(7, pltpu.roll(um, H, 1))


def ssm_scan(u_ref, lam_ref, pw_ref, carry_ref, ini_ref, h_ref, tm, Tc):
    st = Tc + 1
    Lr = lam_ref[0]
    Li = lam_ref[1]
    hr = hi = None
    for j in range(Tc):
        rows = pl.ds(j, 8, stride=st)
        ur = u_ref[0:4, rows, :]
        ui = u_ref[4:8, rows, :]
        if j == 0:
            hr, hi = ur, ui
        else:
            tr_, ti_ = cmul(Lr, Li, hr, hi)
            hr = tr_ + ur
            hi = ti_ + ui
            u_ref[0:4, rows, :] = hr
            u_ref[4:7, rows, :] = hi[0:3]
    sub = lax.broadcasted_iota(jnp.int32, (4, 8, LT), 1)
    er = carry_ref[0]
    ei = carry_ref[1]
    gr = jnp.where(sub == 0, pltpu.roll(er, 1, 1), pltpu.roll(hr, 1, 1))
    gi = jnp.where(sub == 0, pltpu.roll(ei, 1, 1), pltpu.roll(hi, 1, 1))
    for s in range(3):
        sh = 1 << s
        tr_ = jnp.where(sub >= sh, pltpu.roll(gr, sh, 1), 0.0)
        ti_ = jnp.where(sub >= sh, pltpu.roll(gi, sh, 1), 0.0)
        pr_, pi_ = cmul(lam_ref[2 + 2 * s], lam_ref[3 + 2 * s], tr_, ti_)
        gr = gr + pr_
        gi = gi + pi_
    pr_, pi_ = cmul(lam_ref[2], lam_ref[3], gr, gi)
    carry_ref[0] = hr + pr_
    carry_ref[1] = hi + pi_
    ini_ref[0] = gr
    ini_ref[1] = gi
    Pr = pw_ref[0]
    Pi = pw_ref[1]
    for c in range(8):
        ir = ini_ref[0, :, pl.ds(c, 1), :]
        ii = ini_ref[1, :, pl.ds(c, 1), :]
        rows = pl.ds(c * st, Tc)
        vr = u_ref[0:4, rows, :] + (Pr * ir - Pi * ii)
        vi = u_ref[4:7, rows, :] + (Pr[0:3] * ii[0:3] + Pi[0:3] * ir[0:3])
        for k in range(4):
            h_ref[c * Tc:(c + 1) * Tc, k * LT:(k + 1) * LT] = vr[k].astype(bf16)
        for k in range(3):
            h_ref[c * Tc:(c + 1) * Tc, (4 + k) * LT:(5 + k) * LT] = vi[k].astype(bf16)


@jax.jit
def pallas_gated_mix__ssm_conv_s5__glu_gated_geglu__prompt_kernel(
    A_x: jax.Array,
    A_Lambda_re: jax.Array,
    A_Lambda_im: jax.Array,
    A_B_re: jax.Array,
    A_B_im: jax.Array,
    A_C_re: jax.Array,
    A_C_im: jax.Array,
    A_log_dt: jax.Array,
    A_Dskip: jax.Array,
    B_x: jax.Array,
    B_w_gate: jax.Array,
    B_w_up: jax.Array,
    B_w_down: jax.Array,
    gate_w: jax.Array,
):
    Lre, Lim, Bre, Bim, Cre, Cim, log_dt, Dskip = A_Lambda_re, A_Lambda_im, A_B_re, A_B_im, A_C_re, A_C_im, A_log_dt, A_Dskip
    Wg, Wu, Wd = B_w_gate, B_w_up, B_w_down
    tm = 512
    fc = 1792
    tr = "f32"
    interpret = False
    xT = jnp.transpose(A_x[0])
    WdT = jnp.transpose(Wd)
    Tc = tm // 8
    st = Tc + 1

    def kernel(xT_ref, lre_ref, lim_ref, ldt_ref, dsk_ref, gw_ref, bre_ref, bim_ref, cre_ref, cim_ref, wg_ref, wu_ref, wdT_ref,
               o_ref, ccat_ref, lam_ref, pw_ref, dcol_ref, gcol_ref, u_ref, carry_ref, ini_ref, h_ref):
        i = pl.program_id(0)

        @pl.when(i == 0)
        def _():
            prep_params(lre_ref, lim_ref, ldt_ref, dsk_ref, gw_ref, cre_ref, cim_ref, ccat_ref, lam_ref, pw_ref, dcol_ref, gcol_ref, Tc)
            carry_ref[...] = jnp.zeros(carry_ref.shape, f32)

        xTb = xT_ref[...]
        xTf = xTb.astype(f32)
        if tr == "bf16":
            x = xTb.T
        else:
            x = xTf.T.astype(bf16)
        ssm_in(x, bre_ref, bim_ref, u_ref, tm, Tc)
        ssm_scan(u_ref, lam_ref, pw_ref, carry_ref, ini_ref, h_ref, tm, Tc)
        acc = None
        for c in range(F // fc):
            sl = slice(c * fc, (c + 1) * fc)
            g = lax.dot_general(x, wg_ref[:, sl], NN, preferred_element_type=f32)
            u = lax.dot_general(x, wu_ref[:, sl], NN, preferred_element_type=f32)
            hh = (jax.nn.gelu(g, approximate=True) * u).astype(bf16)
            p = lax.dot_general(wdT_ref[:, sl], hh, NT, preferred_element_type=f32)
            acc = p if acc is None else acc + p
        y = lax.dot_general(ccat_ref[...], h_ref[...], NT, preferred_element_type=f32)
        nl = tm // LT
        gcol = jnp.concatenate([gcol_ref[...]] * nl, axis=1)
        dcol = jnp.concatenate([dcol_ref[...]] * nl, axis=1)
        s = jnp.sum(xTf * gcol, axis=0, keepdims=True)
        gt = jax.nn.sigmoid(s)
        o_ref[...] = acc + gt * ((y + xTf * dcol) - acc)

    full = lambda shape: pl.BlockSpec(shape, lambda i: (0,) * len(shape))
    outT = pl.pallas_call(
        kernel,
        grid=(S // tm,),
        in_specs=[pl.BlockSpec((D, tm), lambda i: (0, i)),
                  full((D,)), full((D,)), full((D,)), full((D,)), full((D,)),
                  full((D, D)), full((D, D)), full((D, D)), full((D, D)), full((D, F)), full((D, F)), full((D, F))],
        out_specs=pl.BlockSpec((D, tm), lambda i: (0, i)),
        out_shape=jax.ShapeDtypeStruct((D, S), f32),
        scratch_shapes=[
            pltpu.VMEM((D, 896), bf16),
            pltpu.VMEM((8, 4, 8, LT), f32),
            pltpu.VMEM((2, 4, Tc, LT), f32),
            pltpu.VMEM((D, LT), f32),
            pltpu.VMEM((D, LT), f32),
            pltpu.VMEM((8, 8 * st, LT), f32),
            pltpu.VMEM((2, 4, 8, LT), f32),
            pltpu.VMEM((2, 4, 8, LT), f32),
            pltpu.VMEM((tm, 896), bf16),
        ],
        compiler_params=pltpu.CompilerParams(dimension_semantics=("arbitrary",), vmem_limit_bytes=100 * 2**20),
        interpret=interpret,
    )(xT, Lre, Lim, log_dt, Dskip, gate_w, Bre, Bim, Cre, Cim, Wg, Wu, WdT)
    return jnp.transpose(outT)[None]
```

```python
import jax
import jax.numpy as jnp
from jax import lax
import jax.experimental.pallas as pl
import jax.experimental.pallas.tpu as pltpu

NT = (((1,), (1,)), ((), ()))
NN = (((1,), (0,)), ((), ()))
f32 = jnp.float32
bf16 = jnp.bfloat16
LT = 128
TM = 512
OSPLIT = 4


def _cmul(ar, ai, br, bi):
    return ar * br - ai * bi, ar * bi + ai * br


def _prep_tables(lre_ref, lim_ref, ldt_ref, dsk_ref, gw_ref,
                 coef_ref, lam_ref, pw_ref, dcol_ref, gcol_ref, *, D, Tc):
    nfull = D // LT
    lo = nfull * LT
    lre = lre_ref[...].astype(f32)[None, :]
    lim = lim_ref[...].astype(f32)[None, :]
    dt = jnp.exp(ldt_ref[...].astype(f32)).astype(bf16).astype(f32)[None, :]
    mag = jnp.exp(dt * lre)
    ang = dt * lim
    br = mag * jnp.cos(ang)
    bi = mag * jnp.sin(ang)
    nr = br - 1.0
    ni = bi
    big = jnp.abs(lre) >= jnp.abs(lim)
    num = jnp.where(big, lim, lre)
    den = jnp.where(big, lre, lim)
    r = num / den
    dd = den + num * r
    cr = 2.0 * (jnp.where(big, nr + ni * r, nr * r + ni) / dd)
    ci = 2.0 * (jnp.where(big, ni - nr * r, ni * r - nr) / dd)
    coef_ref[0] = jnp.broadcast_to(cr, (8, D))
    coef_ref[1] = jnp.broadcast_to(ci, (8, D))

    def tiles(v, sign):
        half = jnp.concatenate([v[:, lo:D], sign * v[:, lo:D]], axis=1)
        return jnp.stack([v[:, k * LT:(k + 1) * LT] for k in range(nfull)] + [half], axis=0)

    nk = nfull + 1
    Lr = jnp.broadcast_to(tiles(br, 1.0), (nk, 8, LT))
    Li = jnp.broadcast_to(tiles(bi, -1.0), (nk, 8, LT))
    lam_ref[0] = Lr
    lam_ref[1] = Li
    sub = lax.broadcasted_iota(jnp.int32, (nk, 8, LT), 1) + 1
    qr = jnp.ones((nk, 8, LT), f32)
    qi = jnp.zeros((nk, 8, LT), f32)
    sr, si = Lr, Li
    for b in range(4):
        tr, ti = _cmul(qr, qi, sr, si)
        m = ((sub >> b) & 1) == 1
        qr = jnp.where(m, tr, qr)
        qi = jnp.where(m, ti, qi)
        if b < 3:
            sr, si = _cmul(sr, si, sr, si)
    l8r, l8i = sr, si
    for blk in range(Tc // 8):
        pw_ref[0, :, blk * 8:(blk + 1) * 8, :] = qr
        pw_ref[1, :, blk * 8:(blk + 1) * 8, :] = qi
        if blk + 1 < Tc // 8:
            qr, qi = _cmul(qr, qi, l8r, l8i)
    ar, ai = l8r, l8i
    n = 8
    while n < Tc:
        ar, ai = _cmul(ar, ai, ar, ai)
        n *= 2
    for s in range(3):
        lam_ref[2 + 2 * s] = ar
        lam_ref[3 + 2 * s] = ai
        if s < 2:
            ar, ai = _cmul(ar, ai, ar, ai)
    dsk = dsk_ref[...].astype(f32)[None, :]
    gw = gw_ref[...].astype(f32)[None, :]
    dcol_ref[...] = jnp.broadcast_to(dsk, (LT, D)).T
    gcol_ref[...] = jnp.broadcast_to(gw, (LT, D)).T


def _prep_c(cre_ref, cim_ref, coef_ref, ccat_ref, *, D):
    lo = (D // LT) * LT
    cr = coef_ref[0, 0:1, :]
    ci = coef_ref[1, 0:1, :]
    cre = cre_ref[...].astype(f32)
    cim = cim_ref[...].astype(f32)
    pr = cre * cr - cim * ci
    pi = -(cre * ci + cim * cr)
    ccat_ref[:, 0:lo] = pr[:, 0:lo].astype(bf16)
    ccat_ref[:, lo:lo + LT] = jnp.concatenate([pr[:, lo:D], pi[:, lo:D]], axis=1).astype(bf16)
    ccat_ref[:, lo + LT:2 * lo + LT] = pi[:, 0:lo].astype(bf16)


def _ssm_in(x, bre_ref, bim_ref, u_ref, *, D, Tc):
    nfull = D // LT
    nk = nfull + 1
    lo = nfull * LT
    st = Tc + 1

    def put(k, val):
        for c in range(8):
            u_ref[k, pl.ds(c * st, Tc), :] = val[c * Tc:(c + 1) * Tc, :]

    for k in range(nfull):
        put(k, lax.dot_general(x, bre_ref[k * LT:(k + 1) * LT, :], NT, preferred_element_type=f32))
        put(nk + k, lax.dot_general(x, bim_ref[k * LT:(k + 1) * LT, :], NT, preferred_element_type=f32))
    bm = jnp.concatenate([bre_ref[lo:D, :], bim_ref[lo:D, :]], axis=0)
    um = lax.dot_general(x, bm, NT, preferred_element_type=f32)
    put(nfull, um)
    put(nk + nfull, pltpu.roll(um, LT // 2, 1))


def _scan_local(u_ref, lam_ref, carry_ref, ini_ref, *, D, Tc):
    nfull = D // LT
    nk = nfull + 1
    st = Tc + 1
    Lr = lam_ref[0]
    Li = lam_ref[1]
    hr = hi = None
    for j in range(Tc):
        rows = pl.ds(j, 8, stride=st)
        ur = u_ref[0:nk, rows, :]
        ui = u_ref[nk:2 * nk, rows, :]
        if j == 0:
            hr, hi = ur, ui
        else:
            tr, ti = _cmul(Lr, Li, hr, hi)
            hr = tr + ur
            hi = ti + ui
            u_ref[0:nk, rows, :] = hr
            u_ref[nk:nk + nfull, rows, :] = hi[0:nfull]
    sub = lax.broadcasted_iota(jnp.int32, (nk, 8, LT), 1)
    er = carry_ref[0]
    ei = carry_ref[1]
    gr = jnp.where(sub == 0, pltpu.roll(er, 1, 1), pltpu.roll(hr, 1, 1))
    gi = jnp.where(sub == 0, pltpu.roll(ei, 1, 1), pltpu.roll(hi, 1, 1))
    for s in range(3):
        sh = 1 << s
        tr = jnp.where(sub >= sh, pltpu.roll(gr, sh, 1), 0.0)
        ti = jnp.where(sub >= sh, pltpu.roll(gi, sh, 1), 0.0)
        pr, pi = _cmul(lam_ref[2 + 2 * s], lam_ref[3 + 2 * s], tr, ti)
        gr = gr + pr
        gi = gi + pi
    pr, pi = _cmul(lam_ref[2], lam_ref[3], gr, gi)
    carry_ref[0] = hr + pr
    carry_ref[1] = hi + pi
    ini_ref[0] = gr
    ini_ref[1] = gi


def _scan_fix(u_ref, pw_ref, ini_ref, h_ref, *, D, Tc):
    nfull = D // LT
    nk = nfull + 1
    st = Tc + 1
    Pr = pw_ref[0]
    Pi = pw_ref[1]
    for c in range(8):
        ir = ini_ref[0, :, pl.ds(c, 1), :]
        ii = ini_ref[1, :, pl.ds(c, 1), :]
        rows = pl.ds(c * st, Tc)
        vr = u_ref[0:nk, rows, :] + (Pr * ir - Pi * ii)
        vi = u_ref[nk:nk + nfull, rows, :] + (Pr[0:nfull] * ii[0:nfull] + Pi[0:nfull] * ir[0:nfull])
        for k in range(nk):
            h_ref[c * Tc:(c + 1) * Tc, k * LT:(k + 1) * LT] = vr[k].astype(bf16)
        for k in range(nfull):
            h_ref[c * Tc:(c + 1) * Tc, (nk + k) * LT:(nk + k + 1) * LT] = vi[k].astype(bf16)


def _kernel(xT_hbm, lre_hbm, lim_hbm, ldt_hbm, dsk_hbm, gw_hbm, bre_hbm, bim_hbm, cre_hbm, cim_hbm,
            wg_hbm, wu_hbm, wdT_hbm,
            o_hbm,
            x_s, lre_s, lim_s, ldt_s, dsk_s, gw_s, bre_s, bim_s, cre_s, cim_s, wg_s, wu_s, wdT_s,
            coef_ref, ccat_ref, lam_ref, pw_ref, dcol_ref, gcol_ref, u_ref, carry_ref, ini_ref, h_ref, o_s,
            sems, *, D, F, nt, cuts):
    Tc = TM // 8
    offs = [0] + list(cuts) + [F]
    ng = len(offs) - 1
    SX, SP, SB, SC, SD, SO, SG = 0, nt, nt + 5, nt + 7, nt + 9, nt + 10, 2 * nt + 10

    def cp(src, dst, k):
        return pltpu.make_async_copy(src, dst, sems.at[k])

    def x_copy(i):
        return cp(xT_hbm.at[:, pl.ds(i * TM, TM)], x_s.at[i], SX + i)

    def p_copies():
        pairs = [(lre_hbm, lre_s), (lim_hbm, lim_s), (ldt_hbm, ldt_s), (dsk_hbm, dsk_s), (gw_hbm, gw_s)]
        return [cp(s_, d_, SP + k) for k, (s_, d_) in enumerate(pairs)]

    def b_copies():
        return [cp(bre_hbm, bre_s, SB), cp(bim_hbm, bim_s, SB + 1)]

    def c_copies():
        return [cp(cre_hbm, cre_s, SC), cp(cim_hbm, cim_s, SC + 1)]

    def d_copies():
        return [cp(wdT_hbm, wdT_s, SD)]

    def g_copies(c):
        sl = pl.ds(offs[c], offs[c + 1] - offs[c])
        return [cp(wg_hbm.at[:, sl], wg_s.at[:, sl], SG + 2 * c),
                cp(wu_hbm.at[:, sl], wu_s.at[:, sl], SG + 2 * c + 1)]

    def o_copy(i, lo, n):
        return cp(o_s.at[i, :, pl.ds(lo, n)], o_hbm.at[:, pl.ds(i * TM + lo, n)], SO + i)

    def start(copies):
        for c_ in copies:
            c_.start()

    def wait(copies):
        for c_ in copies:
            c_.wait()

    def load_x(i):
        xTf = x_s[i].astype(f32)
        return xTf, xTf.T.astype(bf16)

    def glu(x, lo, hi):
        g = lax.dot_general(x, wg_s[:, lo:hi], NN, preferred_element_type=f32)
        u = lax.dot_general(x, wu_s[:, lo:hi], NN, preferred_element_type=f32)
        return (jax.nn.gelu(g, approximate=True) * u).astype(bf16)

    def scan():
        _scan_local(u_ref, lam_ref, carry_ref, ini_ref, D=D, Tc=Tc)
        _scan_fix(u_ref, pw_ref, ini_ref, h_ref, D=D, Tc=Tc)

    def finish(i, xTf, hh):
        tq = TM // OSPLIT
        gcol = jnp.concatenate([gcol_ref[...]] * (tq // LT), axis=1)
        dcol = jnp.concatenate([dcol_ref[...]] * (tq // LT), axis=1)
        for q in range(OSPLIT):
            ts = slice(q * tq, (q + 1) * tq)
            b_ = lax.dot_general(wdT_s[...], hh[ts, :], NT, preferred_element_type=f32)
            y_ = lax.dot_general(ccat_ref[...], h_ref[ts, :], NT, preferred_element_type=f32)
            xq = xTf[:, ts]
            gt = jax.nn.sigmoid(jnp.sum(xq * gcol, axis=0, keepdims=True))
            o_s[i, :, ts] = b_ + gt * ((y_ + xq * dcol) - b_)
            o_copy(i, q * tq, tq).start()

    start(p_copies())
    x_copy(0).start()
    start(g_copies(0))
    start(b_copies())
    for c in range(1, ng):
        start(g_copies(c))
    start(d_copies())
    start(c_copies())
    for i in range(1, nt):
        x_copy(i).start()

    wait(p_copies())
    _prep_tables(lre_s, lim_s, ldt_s, dsk_s, gw_s, coef_ref, lam_ref, pw_ref, dcol_ref, gcol_ref, D=D, Tc=Tc)
    carry_ref[...] = jnp.zeros(carry_ref.shape, f32)

    x_copy(0).wait()
    wait(g_copies(0))
    xTf, x = load_x(0)
    hh = [glu(x, offs[0], offs[1])]
    wait(b_copies())
    _ssm_in(x, bre_s, bim_s, u_ref, D=D, Tc=Tc)
    for c in range(1, ng):
        wait(g_copies(c))
        if c == ng - 1:
            wait(d_copies())
            wait(c_copies())
            scan()
            _prep_c(cre_s, cim_s, coef_ref, ccat_ref, D=D)
        hh.append(glu(x, offs[c], offs[c + 1]))
    finish(0, xTf, jnp.concatenate(hh, axis=1))

    def body(i, carry):
        x_copy(i).wait()
        xTf, x = load_x(i)
        _ssm_in(x, bre_s, bim_s, u_ref, D=D, Tc=Tc)
        scan()
        finish(i, xTf, glu(x, 0, F))
        return carry

    lax.fori_loop(1, nt, body, 0)
    for i in range(nt):
        o_copy(i, 0, TM).wait()


@jax.jit
def pallas_gated_mix__ssm_conv_s5__glu_gated_geglu__prompt_kernel(
    A_x: jax.Array,
    A_Lambda_re: jax.Array,
    A_Lambda_im: jax.Array,
    A_B_re: jax.Array,
    A_B_im: jax.Array,
    A_C_re: jax.Array,
    A_C_im: jax.Array,
    A_log_dt: jax.Array,
    A_Dskip: jax.Array,
    B_x: jax.Array,
    B_w_gate: jax.Array,
    B_w_up: jax.Array,
    B_w_down: jax.Array,
    gate_w: jax.Array,
):
    batch, S, D = A_x.shape
    F = B_w_gate.shape[1]
    assert batch == 1 and S % TM == 0 and D == 448 and F % LT == 0
    assert A_B_re.shape == (D, D) and A_C_re.shape == (D, D) and B_w_down.shape == (F, D)
    nt = S // TM
    Tc = TM // 8
    nk = D // LT + 1
    nh = (2 * nk - 1) * LT
    cuts = (128, 1024)

    xT = jnp.transpose(A_x.reshape(S, D))
    wdT = jnp.transpose(B_w_down)

    def kernel(*refs):
        _kernel(*refs, D=D, F=F, nt=nt, cuts=cuts)

    hbm = pl.BlockSpec(memory_space=pltpu.HBM)
    vec = pltpu.VMEM((D,), bf16)
    outT = pl.pallas_call(
        kernel,
        in_specs=[hbm] * 13,
        out_specs=hbm,
        out_shape=jax.ShapeDtypeStruct((D, S), f32),
        scratch_shapes=[
            pltpu.VMEM((nt, D, TM), bf16),
            vec, vec, vec, vec, vec,
            pltpu.VMEM((D, D), bf16), pltpu.VMEM((D, D), bf16),
            pltpu.VMEM((D, D), bf16), pltpu.VMEM((D, D), bf16),
            pltpu.VMEM((D, F), bf16), pltpu.VMEM((D, F), bf16),
            pltpu.VMEM((D, F), bf16),
            pltpu.VMEM((2, 8, D), f32),
            pltpu.VMEM((D, nh), bf16),
            pltpu.VMEM((8, nk, 8, LT), f32),
            pltpu.VMEM((2, nk, Tc, LT), f32),
            pltpu.VMEM((D, LT), f32), pltpu.VMEM((D, LT), f32),
            pltpu.VMEM((2 * nk, 8 * (Tc + 1), LT), f32),
            pltpu.VMEM((2, nk, 8, LT), f32),
            pltpu.VMEM((2, nk, 8, LT), f32),
            pltpu.VMEM((TM, nh), bf16),
            pltpu.VMEM((nt, D, TM), f32),
            pltpu.SemaphoreType.DMA((2 * nt + 10 + 2 * (len(cuts) + 1),)),
        ],
        compiler_params=pltpu.CompilerParams(vmem_limit_bytes=100 * 2**20),
    )(xT, A_Lambda_re, A_Lambda_im, A_log_dt, A_Dskip, gate_w, A_B_re, A_B_im, A_C_re, A_C_im,
      B_w_gate, B_w_up, wdT)
    return jnp.transpose(outT).reshape(batch, S, D)
```

```python
import jax
import jax.numpy as jnp
from jax import lax
import jax.experimental.pallas as pl
import jax.experimental.pallas.tpu as pltpu

NT = (((1,), (1,)), ((), ()))
NN = (((1,), (0,)), ((), ()))
f32 = jnp.float32
bf16 = jnp.bfloat16
LT = 128
TM = 512
OSPLIT = 4
RSPLIT = 4
UCUTS = (256, 768)
SSM_POS = 2


def _cmul(ar, ai, br, bi):
    return ar * br - ai * bi, ar * bi + ai * br


def _prep_tables(lre_ref, lim_ref, ldt_ref, dsk_ref, gw_ref, lam_ref, pw_ref, dcol_ref, gcol_ref, *, D, Tc):
    nfull = D // LT
    lo = nfull * LT
    nk = nfull + 1
    lre = lre_ref[...].astype(f32)[None, :]
    lim = lim_ref[...].astype(f32)[None, :]
    dt = jnp.exp(ldt_ref[...].astype(f32)).astype(bf16).astype(f32)[None, :]
    mag = jnp.exp(dt * lre)
    ang = dt * lim
    br = mag * jnp.cos(ang)
    bi = mag * jnp.sin(ang)
    nr = br - 1.0
    ni = bi
    big = jnp.abs(lre) >= jnp.abs(lim)
    num = jnp.where(big, lim, lre)
    den = jnp.where(big, lre, lim)
    r = num / den
    dd = den + num * r
    cr = 2.0 * (jnp.where(big, nr + ni * r, nr * r + ni) / dd)
    ci = 2.0 * (jnp.where(big, ni - nr * r, ni * r - nr) / dd)

    def tiles(v, s_lo, s_hi):
        half = jnp.concatenate([s_lo * v[:, lo:D], s_hi * v[:, lo:D]], axis=1)
        stacked = jnp.stack([v[:, k * LT:(k + 1) * LT] for k in range(nfull)] + [half], axis=0)
        return jnp.broadcast_to(stacked, (nk, 8, LT))

    Lr = tiles(br, 1.0, 1.0)
    Li = tiles(bi, 1.0, -1.0)
    lam_ref[0] = Lr
    lam_ref[1] = Li
    lam_ref[8] = tiles(cr, 1.0, -1.0)
    lam_ref[9] = tiles(ci, -1.0, -1.0)
    sub = lax.broadcasted_iota(jnp.int32, (nk, 8, LT), 1) + 1
    qr = jnp.ones((nk, 8, LT), f32)
    qi = jnp.zeros((nk, 8, LT), f32)
    sr, si = Lr, Li
    for b in range(4):
        tr, ti = _cmul(qr, qi, sr, si)
        m = ((sub >> b) & 1) == 1
        qr = jnp.where(m, tr, qr)
        qi = jnp.where(m, ti, qi)
        if b < 3:
            sr, si = _cmul(sr, si, sr, si)
    l8r, l8i = sr, si
    for blk in range(Tc // 8):
        pw_ref[0, :, blk * 8:(blk + 1) * 8, :] = qr
        pw_ref[1, :, blk * 8:(blk + 1) * 8, :] = qi
        if blk + 1 < Tc // 8:
            qr, qi = _cmul(qr, qi, l8r, l8i)
    ar, ai = l8r, l8i
    n = 8
    while n < Tc:
        ar, ai = _cmul(ar, ai, ar, ai)
        n *= 2
    for s in range(3):
        lam_ref[2 + 2 * s] = ar
        lam_ref[3 + 2 * s] = ai
        if s < 2:
            ar, ai = _cmul(ar, ai, ar, ai)
    dsk = dsk_ref[...].astype(f32)[None, :]
    gw = gw_ref[...].astype(f32)[None, :]
    dcol_ref[...] = jnp.broadcast_to(dsk, (LT, D)).T
    gcol_ref[...] = jnp.broadcast_to(gw, (LT, D)).T


def _ssm_in(x, bre_ref, bim_ref, u_ref, *, D, Tc):
    nfull = D // LT
    nk = nfull + 1
    lo = nfull * LT
    st = Tc + 1

    def put(k, val):
        for c in range(8):
            u_ref[k, pl.ds(c * st, Tc), :] = val[c * Tc:(c + 1) * Tc, :]

    for k in range(nfull):
        put(k, lax.dot_general(x, bre_ref[k * LT:(k + 1) * LT, :], NT, preferred_element_type=f32))
        put(nk + k, lax.dot_general(x, bim_ref[k * LT:(k + 1) * LT, :], NT, preferred_element_type=f32))
    bm = jnp.concatenate([bre_ref[lo:D, :], bim_ref[lo:D, :]], axis=0)
    um = lax.dot_general(x, bm, NT, preferred_element_type=f32)
    put(nfull, um)
    put(nk + nfull, pltpu.roll(um, LT // 2, 1))


def _scan_local(u_ref, lam_ref, carry_ref, ini_ref, *, D, Tc):
    nk = D // LT + 1
    st = Tc + 1
    Lr = lam_ref[0]
    Li = lam_ref[1]
    hr = hi = None
    for j in range(Tc):
        rows = pl.ds(j, 8, stride=st)
        ur = u_ref[0:nk, rows, :]
        ui = u_ref[nk:2 * nk, rows, :]
        if j == 0:
            hr, hi = ur, ui
        else:
            tr, ti = _cmul(Lr, Li, hr, hi)
            hr = tr + ur
            hi = ti + ui
            u_ref[0:nk, rows, :] = hr
            u_ref[nk:2 * nk, rows, :] = hi
    sub = lax.broadcasted_iota(jnp.int32, (nk, 8, LT), 1)
    er = carry_ref[0]
    ei = carry_ref[1]
    gr = jnp.where(sub == 0, pltpu.roll(er, 1, 1), pltpu.roll(hr, 1, 1))
    gi = jnp.where(sub == 0, pltpu.roll(ei, 1, 1), pltpu.roll(hi, 1, 1))
    for s in range(3):
        sh = 1 << s
        tr = jnp.where(sub >= sh, pltpu.roll(gr, sh, 1), 0.0)
        ti = jnp.where(sub >= sh, pltpu.roll(gi, sh, 1), 0.0)
        pr, pi = _cmul(lam_ref[2 + 2 * s], lam_ref[3 + 2 * s], tr, ti)
        gr = gr + pr
        gi = gi + pi
    pr, pi = _cmul(lam_ref[2], lam_ref[3], gr, gi)
    carry_ref[0] = hr + pr
    carry_ref[1] = hi + pi
    ini_ref[0] = gr
    ini_ref[1] = gi


def _scan_fix(u_ref, lam_ref, pw_ref, ini_ref, h_ref, *, D, Tc):
    nfull = D // LT
    nk = nfull + 1
    st = Tc + 1
    Pr = pw_ref[0]
    Pi = pw_ref[1]
    Cr = lam_ref[8, :, 0:1, :]
    Ci = lam_ref[9, :, 0:1, :]
    for c in range(8):
        ir = ini_ref[0, :, pl.ds(c, 1), :]
        ii = ini_ref[1, :, pl.ds(c, 1), :]
        rows = pl.ds(c * st, Tc)
        vr = u_ref[0:nk, rows, :] + (Pr * ir - Pi * ii)
        vi = u_ref[nk:2 * nk, rows, :] + (Pr * ii + Pi * ir)
        sr = Cr[0:nfull] * vr[0:nfull] - Ci[0:nfull] * vi[0:nfull]
        si = (-Cr[0:nfull]) * vi[0:nfull] - Ci[0:nfull] * vr[0:nfull]
        sm = Cr[nfull] * vr[nfull] + Ci[nfull] * vi[nfull]
        trows = slice(c * Tc, (c + 1) * Tc)
        for k in range(nfull):
            h_ref[trows, k * LT:(k + 1) * LT] = sr[k].astype(bf16)
            h_ref[trows, (nk + k) * LT:(nk + k + 1) * LT] = si[k].astype(bf16)
        h_ref[trows, nfull * LT:nk * LT] = sm.astype(bf16)


def _kernel(xT_hbm, lre_hbm, lim_hbm, ldt_hbm, dsk_hbm, gw_hbm, bre_hbm, bim_hbm, cre_hbm, cim_hbm,
            wg_hbm, wu_hbm, wdT_hbm,
            o_hbm,
            x_s, lre_s, lim_s, ldt_s, dsk_s, gw_s, bre_s, bim_s, cre_s, cim_s, wg_s, wu_s, wdT_s,
            lam_ref, pw_ref, dcol_ref, gcol_ref, u_ref, carry_ref, ini_ref, h_ref, o_s,
            sems, *, D, F, nt):
    Tc = TM // 8
    lo = (D // LT) * LT
    uo = [0] + list(UCUTS) + [F]
    nu = len(uo) - 1
    SX, SP, SB, SC, SD, SO, SW = 0, nt, nt + 5, nt + 7, nt + 9, nt + 10, 2 * nt + 10

    def cp(src, dst, k):
        return pltpu.make_async_copy(src, dst, sems.at[k])

    def x_copy(i):
        return cp(xT_hbm.at[:, pl.ds(i * TM, TM)], x_s.at[i], SX + i)

    def p_copies():
        pairs = [(lre_hbm, lre_s), (lim_hbm, lim_s), (ldt_hbm, ldt_s), (dsk_hbm, dsk_s), (gw_hbm, gw_s)]
        return [cp(s_, d_, SP + k) for k, (s_, d_) in enumerate(pairs)]

    def b_copies():
        return [cp(bre_hbm, bre_s, SB), cp(bim_hbm, bim_s, SB + 1)]

    def c_copies():
        return [cp(cre_hbm, cre_s, SC), cp(cim_hbm, cim_s, SC + 1)]

    def d_copies():
        return [cp(wdT_hbm, wdT_s, SD)]

    def w_copies(k, which):
        sl = pl.ds(uo[k], uo[k + 1] - uo[k])
        src, dst = (wg_hbm, wg_s) if which == 0 else (wu_hbm, wu_s)
        return [cp(src.at[:, sl], dst.at[:, sl], SW + 2 * k + which)]

    def o_copy(i, r0, nr, t0, nt_):
        return cp(o_s.at[i, pl.ds(r0, nr), pl.ds(t0, nt_)],
                  o_hbm.at[pl.ds(r0, nr), pl.ds(i * TM + t0, nt_)], SO + i)

    def start(copies):
        for c_ in copies:
            c_.start()

    def wait(copies):
        for c_ in copies:
            c_.wait()

    start(p_copies())
    x_copy(0).start()
    for k in range(nu):
        if k == SSM_POS:
            start(b_copies())
        start(w_copies(k, 0))
        start(w_copies(k, 1))
    start(c_copies())
    start(d_copies())
    for i in range(1, nt):
        x_copy(i).start()

    wait(p_copies())
    _prep_tables(lre_s, lim_s, ldt_s, dsk_s, gw_s, lam_ref, pw_ref, dcol_ref, gcol_ref, D=D, Tc=Tc)
    carry_ref[...] = jnp.zeros(carry_ref.shape, f32)

    def tile(i, carry):
        def first_use(copies):
            pl.when(i == 0)(lambda: wait(copies()))

        x_copy(i).wait()
        xTf = x_s[i].astype(f32)
        x = xTf.T.astype(bf16)
        hh = []
        for k in range(nu):
            if k == SSM_POS:
                first_use(b_copies)
                _ssm_in(x, bre_s, bim_s, u_ref, D=D, Tc=Tc)
                _scan_local(u_ref, lam_ref, carry_ref, ini_ref, D=D, Tc=Tc)
                _scan_fix(u_ref, lam_ref, pw_ref, ini_ref, h_ref, D=D, Tc=Tc)
            cols = slice(uo[k], uo[k + 1])
            first_use(lambda k=k: w_copies(k, 0))
            g = lax.dot_general(x, wg_s[:, cols], NN, preferred_element_type=f32)
            first_use(lambda k=k: w_copies(k, 1))
            u = lax.dot_general(x, wu_s[:, cols], NN, preferred_element_type=f32)
            hh.append((jax.nn.gelu(g, approximate=True) * u).astype(bf16))
        hh = jnp.concatenate(hh, axis=1)
        first_use(c_copies)
        first_use(d_copies)
        cre = cre_s[...]
        cim = cim_s[...]
        cmix = jnp.concatenate([cre[:, lo:D], cim[:, lo:D]], axis=1)
        ccat = jnp.concatenate([cre[:, 0:lo], cmix, cim[:, 0:lo]], axis=1)
        tq = TM // OSPLIT
        gcol = jnp.concatenate([gcol_ref[...]] * (tq // LT), axis=1)
        dcol = jnp.concatenate([dcol_ref[...]] * (tq // LT), axis=1)
        for q in range(OSPLIT):
            ts = slice(q * tq, (q + 1) * tq)
            b_ = lax.dot_general(wdT_s[...], hh[ts, :], NT, preferred_element_type=f32)
            y_ = lax.dot_general(ccat, h_ref[ts, :], NT, preferred_element_type=f32)
            xq = xTf[:, ts]
            gt = jax.nn.sigmoid(jnp.sum(xq * gcol, axis=0, keepdims=True))
            res = b_ + gt * ((y_ + xq * dcol) - b_)
            nr = RSPLIT if q == OSPLIT - 1 else 1
            rr = D // nr
            for r in range(nr):
                o_s[i, r * rr:(r + 1) * rr, ts] = res[r * rr:(r + 1) * rr, :]
                o_copy(i, r * rr, rr, q * tq, tq).start()
        return carry

    lax.fori_loop(0, nt, tile, 0)
    for i in range(nt):
        o_copy(i, 0, D, 0, TM).wait()


@jax.jit
def pallas_gated_mix__ssm_conv_s5__glu_gated_geglu__prompt_kernel(
    A_x: jax.Array,
    A_Lambda_re: jax.Array,
    A_Lambda_im: jax.Array,
    A_B_re: jax.Array,
    A_B_im: jax.Array,
    A_C_re: jax.Array,
    A_C_im: jax.Array,
    A_log_dt: jax.Array,
    A_Dskip: jax.Array,
    B_x: jax.Array,
    B_w_gate: jax.Array,
    B_w_up: jax.Array,
    B_w_down: jax.Array,
    gate_w: jax.Array,
):
    batch, S, D = A_x.shape
    F = B_w_gate.shape[1]
    assert batch == 1 and S % TM == 0 and D == 448 and F == 1792
    assert A_B_re.shape == (D, D) and A_C_re.shape == (D, D) and B_w_down.shape == (F, D)
    nt = S // TM
    Tc = TM // 8
    nk = D // LT + 1
    nh = (2 * nk - 1) * LT

    xT = jnp.transpose(A_x.reshape(S, D))
    wdT = jnp.transpose(B_w_down)

    def kernel(*refs):
        _kernel(*refs, D=D, F=F, nt=nt)

    hbm = pl.BlockSpec(memory_space=pltpu.HBM)
    vec = pltpu.VMEM((D,), bf16)
    outT = pl.pallas_call(
        kernel,
        in_specs=[hbm] * 13,
        out_specs=hbm,
        out_shape=jax.ShapeDtypeStruct((D, S), f32),
        scratch_shapes=[
            pltpu.VMEM((nt, D, TM), bf16),
            vec, vec, vec, vec, vec,
            pltpu.VMEM((D, D), bf16), pltpu.VMEM((D, D), bf16),
            pltpu.VMEM((D, D), bf16), pltpu.VMEM((D, D), bf16),
            pltpu.VMEM((D, F), bf16), pltpu.VMEM((D, F), bf16),
            pltpu.VMEM((D, F), bf16),
            pltpu.VMEM((10, nk, 8, LT), f32),
            pltpu.VMEM((2, nk, Tc, LT), f32),
            pltpu.VMEM((D, LT), f32), pltpu.VMEM((D, LT), f32),
            pltpu.VMEM((2 * nk, 8 * (Tc + 1), LT), f32),
            pltpu.VMEM((2, nk, 8, LT), f32),
            pltpu.VMEM((2, nk, 8, LT), f32),
            pltpu.VMEM((TM, nh), bf16),
            pltpu.VMEM((nt, D, TM), f32),
            pltpu.SemaphoreType.DMA((2 * nt + 10 + 2 * (len(UCUTS) + 1),)),
        ],
        compiler_params=pltpu.CompilerParams(
            vmem_limit_bytes=100 * 2**20,
            flags={"XLA_TPU_RESCHEDULE_DMA_DONES": True},
        ),
    )(xT, A_Lambda_re, A_Lambda_im, A_log_dt, A_Dskip, gate_w, A_B_re, A_B_im, A_C_re, A_C_im,
      B_w_gate, B_w_up, wdT)
    return jnp.transpose(outT).reshape(batch, S, D)
```

```python
import jax
import jax.numpy as jnp
from jax import lax
import jax.experimental.pallas as pl
import jax.experimental.pallas.tpu as pltpu

NT = (((1,), (1,)), ((), ()))
NN = (((1,), (0,)), ((), ()))
f32 = jnp.float32
bf16 = jnp.bfloat16
LT = 128
TM = 512
OSPLIT = 4
RSPLIT = 8
UCUTS = (256, 768)
SSM_POS = 2


def _cmul(ar, ai, br, bi):
    return ar * br - ai * bi, ar * bi + ai * br


def _prep_tables(lre_ref, lim_ref, ldt_ref, dsk_ref, gw_ref, lam_ref, pw_ref, dcol_ref, gcol_ref, *, D, Tc):
    nfull = D // LT
    lo = nfull * LT
    nk = nfull + 1
    lre = lre_ref[...].astype(f32)[None, :]
    lim = lim_ref[...].astype(f32)[None, :]
    dt = jnp.exp(ldt_ref[...].astype(f32)).astype(bf16).astype(f32)[None, :]
    mag = jnp.exp(dt * lre)
    ang = dt * lim
    br = mag * jnp.cos(ang)
    bi = mag * jnp.sin(ang)
    nr = br - 1.0
    ni = bi
    big = jnp.abs(lre) >= jnp.abs(lim)
    num = jnp.where(big, lim, lre)
    den = jnp.where(big, lre, lim)
    r = num / den
    dd = den + num * r
    cr = 2.0 * (jnp.where(big, nr + ni * r, nr * r + ni) / dd)
    ci = 2.0 * (jnp.where(big, ni - nr * r, ni * r - nr) / dd)

    def tiles(v, s_lo, s_hi):
        half = jnp.concatenate([s_lo * v[:, lo:D], s_hi * v[:, lo:D]], axis=1)
        stacked = jnp.stack([v[:, k * LT:(k + 1) * LT] for k in range(nfull)] + [half], axis=0)
        return jnp.broadcast_to(stacked, (nk, 8, LT))

    Lr = tiles(br, 1.0, 1.0)
    Li = tiles(bi, 1.0, -1.0)
    lam_ref[0] = Lr
    lam_ref[1] = Li
    lam_ref[8] = tiles(cr, 1.0, -1.0)
    lam_ref[9] = tiles(ci, -1.0, -1.0)
    sub = lax.broadcasted_iota(jnp.int32, (nk, 8, LT), 1) + 1
    qr = jnp.ones((nk, 8, LT), f32)
    qi = jnp.zeros((nk, 8, LT), f32)
    sr, si = Lr, Li
    for b in range(4):
        tr, ti = _cmul(qr, qi, sr, si)
        m = ((sub >> b) & 1) == 1
        qr = jnp.where(m, tr, qr)
        qi = jnp.where(m, ti, qi)
        if b < 3:
            sr, si = _cmul(sr, si, sr, si)
    l8r, l8i = sr, si
    for blk in range(Tc // 8):
        pw_ref[0, :, blk * 8:(blk + 1) * 8, :] = qr
        pw_ref[1, :, blk * 8:(blk + 1) * 8, :] = qi
        if blk + 1 < Tc // 8:
            qr, qi = _cmul(qr, qi, l8r, l8i)
    ar, ai = l8r, l8i
    n = 8
    while n < Tc:
        ar, ai = _cmul(ar, ai, ar, ai)
        n *= 2
    for s in range(3):
        lam_ref[2 + 2 * s] = ar
        lam_ref[3 + 2 * s] = ai
        if s < 2:
            ar, ai = _cmul(ar, ai, ar, ai)
    dsk = dsk_ref[...].astype(f32)[None, :]
    gw = gw_ref[...].astype(f32)[None, :]
    dcol_ref[...] = jnp.broadcast_to(dsk, (LT, D)).T
    gcol_ref[...] = jnp.broadcast_to(gw, (LT, D)).T


def _ssm_in(x, bre_ref, bim_ref, u_ref, *, D, Tc):
    nfull = D // LT
    nk = nfull + 1
    lo = nfull * LT
    st = Tc + 1

    def put(k, val):
        for c in range(8):
            u_ref[k, pl.ds(c * st, Tc), :] = val[c * Tc:(c + 1) * Tc, :]

    for k in range(nfull):
        put(k, lax.dot_general(x, bre_ref[k * LT:(k + 1) * LT, :], NT, preferred_element_type=f32))
        put(nk + k, lax.dot_general(x, bim_ref[k * LT:(k + 1) * LT, :], NT, preferred_element_type=f32))
    bm = jnp.concatenate([bre_ref[lo:D, :], bim_ref[lo:D, :]], axis=0)
    um = lax.dot_general(x, bm, NT, preferred_element_type=f32)
    put(nfull, um)
    put(nk + nfull, pltpu.roll(um, LT // 2, 1))


def _scan_local(u_ref, lam_ref, carry_ref, ini_ref, *, D, Tc):
    nk = D // LT + 1
    st = Tc + 1
    Lr = lam_ref[0]
    Li = lam_ref[1]
    hr = hi = None
    for j in range(Tc):
        rows = pl.ds(j, 8, stride=st)
        ur = u_ref[0:nk, rows, :]
        ui = u_ref[nk:2 * nk, rows, :]
        if j == 0:
            hr, hi = ur, ui
        else:
            tr, ti = _cmul(Lr, Li, hr, hi)
            hr = tr + ur
            hi = ti + ui
            u_ref[0:nk, rows, :] = hr
            u_ref[nk:2 * nk, rows, :] = hi
    sub = lax.broadcasted_iota(jnp.int32, (nk, 8, LT), 1)
    er = carry_ref[0]
    ei = carry_ref[1]
    gr = jnp.where(sub == 0, pltpu.roll(er, 1, 1), pltpu.roll(hr, 1, 1))
    gi = jnp.where(sub == 0, pltpu.roll(ei, 1, 1), pltpu.roll(hi, 1, 1))
    for s in range(3):
        sh = 1 << s
        tr = jnp.where(sub >= sh, pltpu.roll(gr, sh, 1), 0.0)
        ti = jnp.where(sub >= sh, pltpu.roll(gi, sh, 1), 0.0)
        pr, pi = _cmul(lam_ref[2 + 2 * s], lam_ref[3 + 2 * s], tr, ti)
        gr = gr + pr
        gi = gi + pi
    pr, pi = _cmul(lam_ref[2], lam_ref[3], gr, gi)
    carry_ref[0] = hr + pr
    carry_ref[1] = hi + pi
    ini_ref[0] = gr
    ini_ref[1] = gi


def _scan_fix(u_ref, lam_ref, pw_ref, ini_ref, h_ref, *, D, Tc):
    nfull = D // LT
    nk = nfull + 1
    st = Tc + 1
    Pr = pw_ref[0]
    Pi = pw_ref[1]
    Cr = lam_ref[8, :, 0:1, :]
    Ci = lam_ref[9, :, 0:1, :]
    for c in range(8):
        ir = ini_ref[0, :, pl.ds(c, 1), :]
        ii = ini_ref[1, :, pl.ds(c, 1), :]
        rows = pl.ds(c * st, Tc)
        vr = u_ref[0:nk, rows, :] + (Pr * ir - Pi * ii)
        vi = u_ref[nk:2 * nk, rows, :] + (Pr * ii + Pi * ir)
        sr = Cr[0:nfull] * vr[0:nfull] - Ci[0:nfull] * vi[0:nfull]
        si = (-Cr[0:nfull]) * vi[0:nfull] - Ci[0:nfull] * vr[0:nfull]
        sm = Cr[nfull] * vr[nfull] + Ci[nfull] * vi[nfull]
        trows = slice(c * Tc, (c + 1) * Tc)
        for k in range(nfull):
            h_ref[trows, k * LT:(k + 1) * LT] = sr[k].astype(bf16)
            h_ref[trows, (nk + k) * LT:(nk + k + 1) * LT] = si[k].astype(bf16)
        h_ref[trows, nfull * LT:nk * LT] = sm.astype(bf16)


def _kernel(xT_hbm, lre_hbm, lim_hbm, ldt_hbm, dsk_hbm, gw_hbm, bre_hbm, bim_hbm, cre_hbm, cim_hbm,
            wg_hbm, wu_hbm, wdT_hbm,
            o_hbm,
            x_s, lre_s, lim_s, ldt_s, dsk_s, gw_s, bre_s, bim_s, cre_s, cim_s, wg_s, wu_s, wdT_s,
            lam_ref, pw_ref, dcol_ref, gcol_ref, u_ref, carry_ref, ini_ref, h_ref, o_s,
            sems, *, D, F, nt):
    Tc = TM // 8
    lo = (D // LT) * LT
    uo = [0] + list(UCUTS) + [F]
    nu = len(uo) - 1
    SX, SP, SB, SC, SD, SO, SW = 0, nt, nt + 5, nt + 7, nt + 9, nt + 10, 2 * nt + 10

    def cp(src, dst, k):
        return pltpu.make_async_copy(src, dst, sems.at[k])

    def x_copy(i):
        return cp(xT_hbm.at[:, pl.ds(i * TM, TM)], x_s.at[i], SX + i)

    def p_copies():
        pairs = [(lre_hbm, lre_s), (lim_hbm, lim_s), (ldt_hbm, ldt_s), (dsk_hbm, dsk_s), (gw_hbm, gw_s)]
        return [cp(s_, d_, SP + k) for k, (s_, d_) in enumerate(pairs)]

    def b_copies():
        return [cp(bre_hbm, bre_s, SB), cp(bim_hbm, bim_s, SB + 1)]

    def c_copies():
        return [cp(cre_hbm, cre_s, SC), cp(cim_hbm, cim_s, SC + 1)]

    def d_copies():
        return [cp(wdT_hbm, wdT_s, SD)]

    def w_copies(k, which):
        sl = pl.ds(uo[k], uo[k + 1] - uo[k])
        src, dst = (wg_hbm, wg_s) if which == 0 else (wu_hbm, wu_s)
        return [cp(src.at[:, sl], dst.at[:, sl], SW + 2 * k + which)]

    def o_copy(i, r0, nr, t0, nt_):
        return cp(o_s.at[i, pl.ds(r0, nr), pl.ds(t0, nt_)],
                  o_hbm.at[pl.ds(r0, nr), pl.ds(i * TM + t0, nt_)], SO + i)

    def start(copies):
        for c_ in copies:
            c_.start()

    def wait(copies):
        for c_ in copies:
            c_.wait()

    start(p_copies())
    x_copy(0).start()
    for k in range(nu):
        if k == SSM_POS:
            start(b_copies())
        start(w_copies(k, 0))
        start(w_copies(k, 1))
    start(c_copies())
    start(d_copies())
    for i in range(1, nt):
        x_copy(i).start()

    wait(p_copies())
    _prep_tables(lre_s, lim_s, ldt_s, dsk_s, gw_s, lam_ref, pw_ref, dcol_ref, gcol_ref, D=D, Tc=Tc)
    carry_ref[...] = jnp.zeros(carry_ref.shape, f32)

    def tile(i, carry):
        def first_use(copies):
            pl.when(i == 0)(lambda: wait(copies()))

        x_copy(i).wait()
        x = x_s[i].astype(f32).T.astype(bf16)
        hh = []
        for k in range(nu):
            if k == SSM_POS:
                first_use(b_copies)
                _ssm_in(x, bre_s, bim_s, u_ref, D=D, Tc=Tc)
                _scan_local(u_ref, lam_ref, carry_ref, ini_ref, D=D, Tc=Tc)
                _scan_fix(u_ref, lam_ref, pw_ref, ini_ref, h_ref, D=D, Tc=Tc)
            cols = slice(uo[k], uo[k + 1])
            first_use(lambda k=k: w_copies(k, 0))
            g = lax.dot_general(x, wg_s[:, cols], NN, preferred_element_type=f32)
            first_use(lambda k=k: w_copies(k, 1))
            u = lax.dot_general(x, wu_s[:, cols], NN, preferred_element_type=f32)
            hh.append((jax.nn.gelu(g, approximate=True) * u).astype(bf16))
        hh = jnp.concatenate(hh, axis=1)
        first_use(c_copies)
        first_use(d_copies)
        cre = cre_s[...]
        cim = cim_s[...]
        cmix = jnp.concatenate([cre[:, lo:D], cim[:, lo:D]], axis=1)
        ccat = jnp.concatenate([cre[:, 0:lo], cmix, cim[:, 0:lo]], axis=1)
        tq = TM // OSPLIT
        gcol = jnp.concatenate([gcol_ref[...]] * (tq // LT), axis=1)
        dcol = jnp.concatenate([dcol_ref[...]] * (tq // LT), axis=1)
        for q in range(OSPLIT):
            ts = slice(q * tq, (q + 1) * tq)
            y_ = lax.dot_general(ccat, h_ref[ts, :], NT, preferred_element_type=f32)
            b_ = lax.dot_general(wdT_s[...], hh[ts, :], NT, preferred_element_type=f32)
            xq = x_s[i, :, ts].astype(f32)
            gt = jax.nn.sigmoid(jnp.sum(xq * gcol, axis=0, keepdims=True))
            res = b_ + gt * ((y_ + xq * dcol) - b_)
            nr = RSPLIT if q == OSPLIT - 1 else 1
            rr = D // nr
            for r in range(nr):
                o_s[i, r * rr:(r + 1) * rr, ts] = res[r * rr:(r + 1) * rr, :]
                o_copy(i, r * rr, rr, q * tq, tq).start()
        return carry

    lax.fori_loop(0, nt, tile, 0)
    for i in range(nt):
        o_copy(i, 0, D, 0, TM).wait()


@jax.jit
def pallas_gated_mix__ssm_conv_s5__glu_gated_geglu__prompt_kernel(
    A_x: jax.Array,
    A_Lambda_re: jax.Array,
    A_Lambda_im: jax.Array,
    A_B_re: jax.Array,
    A_B_im: jax.Array,
    A_C_re: jax.Array,
    A_C_im: jax.Array,
    A_log_dt: jax.Array,
    A_Dskip: jax.Array,
    B_x: jax.Array,
    B_w_gate: jax.Array,
    B_w_up: jax.Array,
    B_w_down: jax.Array,
    gate_w: jax.Array,
):
    batch, S, D = A_x.shape
    F = B_w_gate.shape[1]
    assert batch == 1 and S % TM == 0 and D == 448 and F == 1792
    assert A_B_re.shape == (D, D) and A_C_re.shape == (D, D) and B_w_down.shape == (F, D)
    nt = S // TM
    Tc = TM // 8
    nk = D // LT + 1
    nh = (2 * nk - 1) * LT

    xT = jnp.transpose(A_x.reshape(S, D))
    wdT = jnp.transpose(B_w_down)

    def kernel(*refs):
        _kernel(*refs, D=D, F=F, nt=nt)

    hbm = pl.BlockSpec(memory_space=pltpu.HBM)
    vec = pltpu.VMEM((D,), bf16)
    outT = pl.pallas_call(
        kernel,
        in_specs=[hbm] * 13,
        out_specs=hbm,
        out_shape=jax.ShapeDtypeStruct((D, S), f32),
        scratch_shapes=[
            pltpu.VMEM((nt, D, TM), bf16),
            vec, vec, vec, vec, vec,
            pltpu.VMEM((D, D), bf16), pltpu.VMEM((D, D), bf16),
            pltpu.VMEM((D, D), bf16), pltpu.VMEM((D, D), bf16),
            pltpu.VMEM((D, F), bf16), pltpu.VMEM((D, F), bf16),
            pltpu.VMEM((D, F), bf16),
            pltpu.VMEM((10, nk, 8, LT), f32),
            pltpu.VMEM((2, nk, Tc, LT), f32),
            pltpu.VMEM((D, LT), f32), pltpu.VMEM((D, LT), f32),
            pltpu.VMEM((2 * nk, 8 * (Tc + 1), LT), f32),
            pltpu.VMEM((2, nk, 8, LT), f32),
            pltpu.VMEM((2, nk, 8, LT), f32),
            pltpu.VMEM((TM, nh), bf16),
            pltpu.VMEM((nt, D, TM), f32),
            pltpu.SemaphoreType.DMA((2 * nt + 10 + 2 * (len(UCUTS) + 1),)),
        ],
        compiler_params=pltpu.CompilerParams(
            vmem_limit_bytes=100 * 2**20,
            flags={"XLA_TPU_RESCHEDULE_DMA_DONES": True},
        ),
    )(xT, A_Lambda_re, A_Lambda_im, A_log_dt, A_Dskip, gate_w, A_B_re, A_B_im, A_C_re, A_C_im,
      B_w_gate, B_w_up, wdT)
    return jnp.transpose(outT).reshape(batch, S, D)
```
